```python
import os as _os
_os.environ.setdefault("JAX_PLATFORMS", "cpu")
import jax
import jax.numpy as jnp

def _softmax(x, axis=-1):
    return jax.nn.softmax(x, axis=axis)
def _gelu(x):
    return jax.nn.gelu(x, approximate=True)
def _silu(x):
    return jax.nn.silu(x)
def _sigmoid(x):
    return jax.nn.sigmoid(x)
def _layernorm(x, axis=-1, eps=1e-5):
    m = jnp.mean(x, axis=axis, keepdims=True)
    v = jnp.var(x, axis=axis, keepdims=True)
    return (x - m) / jnp.sqrt(v + eps)
def _scatter_add(tgt, idx, src, axis=0):
    return tgt.at[idx].add(src)
def _segment_sum(src, seg, n):
    return jax.ops.segment_sum(src, seg, n)
class _Rng:
    def __init__(self, key):
        self._k = key
    def _next(self):
        self._k, sub = jax.random.split(self._k)
        return sub
    def normal(self, shape):
        return jax.random.normal(self._next(), shape, dtype=jnp.bfloat16)
    def randint(self, lo, hi, shape):
        return jax.random.randint(self._next(), shape, lo, hi, dtype=jnp.int32)
    def uniform(self, shape, lo=0.0, hi=1.0):
        return jax.random.uniform(self._next(), shape, jnp.bfloat16, lo, hi)
    def permutation(self, n):
        return jax.random.permutation(self._next(), n)


kernel_name = 'sequential_preLN__linear_attn_block__dense_activation_squared_relu__prompt'

def setup_inputs():
    _rng = _Rng(jax.random.key(int.from_bytes(__import__("os").urandom(4), "little")))
    _w = (lambda a: (lambda t: t.astype(jnp.bfloat16) if jnp.issubdtype(t.dtype, jnp.floating) else t)(jnp.asarray(a)))
    def _A_setup():
        B, S, D = 1, 2048, 576
        return {
            "x": _w((lambda *s: _rng.normal(s) * 0.05)(B, S, D)),
            "wqkv": _w((lambda *s: _rng.normal(s) * 0.1)(D, 3 * D)),
            "wo": _w((lambda *s: _rng.normal(s) * 0.05)(D, D)),
        }
    _A_in = _A_setup()

    def _B_setup():
        B, S, D, F = 1, 2048, 576, 4608
        return {
            "x": _w((lambda *s: _rng.normal(s) * 0.05)(B, S, D)),
            "w1": _w((lambda *s: _rng.normal(s) * 0.05)(D, F)),
            "b1": _w((lambda *s: _rng.normal(s) * 0.05)(F)),
            "w2": _w((lambda *s: _rng.normal(s) * 0.05)(F, D)),
            "b2": _w((lambda *s: _rng.normal(s) * 0.05)(D)),
        }
    _B_in = _B_setup()

    return {
        "A_x": _A_in["x"],
        "A_wqkv": _A_in["wqkv"],
        "A_wo": _A_in["wo"],
        "B_x": _B_in["x"],
        "B_w1": _B_in["w1"],
        "B_b1": _B_in["b1"],
        "B_w2": _B_in["w2"],
        "B_b2": _B_in["b2"],
    }

def reference(A_x, A_wqkv, A_wo, B_x, B_w1, B_b1, B_w2, B_b2):
    def _A_ref(x, wqkv, wo):
        B, S, D = x.shape
        H = 32; Dh = D // H
        qkv = (lambda x, *d: x.transpose(*d))((x @ wqkv).reshape(B, S, 3, H, Dh), 2, 0, 3, 1, 4)
        q, k, v = qkv[0], qkv[1], qkv[2]
        phi = lambda t: jnp.where(t > 0, t + 1, jnp.exp(t)) + 1e-6
        pq, pk = phi(q), phi(k)
        kv = jnp.einsum("bhsd,bhse->bhde", pk, v)
        z = jnp.einsum("bhsd->bhd", pk)
        num = jnp.einsum("bhqd,bhde->bhqe", pq, kv)
        den = jnp.einsum("bhqd,bhd->bhq", pq, z)[..., None] + 1e-6
        o = num / den
        return (lambda x, *d: x.transpose(*d))(o, 0, 2, 1, 3).reshape(B, S, D) @ wo

    def _B_ref(x, w1, b1, w2, b2):
        h = jnp.einsum("bsd,df->bsf", x, w1) + b1
        zero = jnp.zeros_like(h)
        r = jnp.where(h > zero, h, zero)
        h = r * r
        out = jnp.einsum("bsf,fd->bsd", h, w2) + b2
        return out

    x = A_x
    h = x + _A_ref(_layernorm(x, axis=-1), A_wqkv, A_wo)
    h2 = h + _B_ref(_layernorm(h, axis=-1), B_w1, B_b1, B_w2, B_b2)
    return h2
```

```python
import functools
import jax
import jax.numpy as jnp
from jax import lax
import jax.experimental.pallas as pl
import jax.experimental.pallas.tpu as pltpu

S, D, F, H = 2048, 576, 4608, 32
DH = D // H
TN1 = 512
TN2 = 512
FC = 512
EPS = 1e-5
f32 = jnp.float32
bf16 = jnp.bfloat16
NT = (((1,), (1,)), ((), ()))


def _lnT(x):
    mu = jnp.mean(x, axis=0, keepdims=True)
    xc = x - mu
    var = jnp.mean(xc * xc, axis=0, keepdims=True)
    return xc * lax.rsqrt(var + EPS)


def _phi(t):
    return jnp.where(t > 0, t + 1.0, jnp.exp(t)) + 1e-6


def _head_of(idx_f32):
    return jnp.floor((idx_f32 + 0.5) * (1.0 / DH))


def _kernel(xT_hbm, wqkv_hbm, wo_hbm, w1_hbm, b1_ref, w2T_hbm, b2_ref, oT_hbm,
            xT_v, wqkv_v, wo_v, w1_v, w2T_v, wqkvT_v, pqT_v, kv_acc, z_acc, mT_v, zc_v, e_v, b2c_v, oT_v, sems):
    cp_x = pltpu.make_async_copy(xT_hbm, xT_v, sems.at[0])
    cp_wqkv = pltpu.make_async_copy(wqkv_hbm, wqkv_v, sems.at[1])
    cp_wo = pltpu.make_async_copy(wo_hbm, wo_v, sems.at[2])
    cp_w1 = pltpu.make_async_copy(w1_hbm, w1_v, sems.at[3])
    cp_w2 = pltpu.make_async_copy(w2T_hbm, w2T_v, sems.at[4])
    cp_wqkv.start()
    cp_x.start()
    cp_wqkv.wait()
    cp_wo.start()
    cp_w1.start()
    cp_w2.start()

    wqkvT_v[...] = wqkv_v[...].astype(f32).T.astype(bf16)
    kv_acc[...] = jnp.zeros_like(kv_acc)
    z_acc[...] = jnp.zeros_like(z_acc)
    b2c_v[...] = jnp.broadcast_to(b2_ref[...].astype(f32), (128, D)).T
    cp_x.wait()

    def p1(i, c):
        c0 = pl.multiple_of(i * TN1, TN1)
        x = xT_v[:, pl.ds(c0, TN1)].astype(f32)
        xln = _lnT(x).astype(bf16)
        qkvT = jnp.dot(wqkvT_v[...], xln, preferred_element_type=f32)
        pqT_v[:, pl.ds(c0, TN1)] = _phi(qkvT[0:D]).astype(bf16)
        pkT = _phi(qkvT[D:2 * D])
        vT = qkvT[2 * D:3 * D].astype(bf16)
        zs = pkT[:, 0:128]
        for j in range(1, TN1 // 128):
            zs = zs + pkT[:, j * 128:(j + 1) * 128]
        z_acc[...] += zs
        kv_acc[...] += lax.dot_general(pkT.astype(bf16), vT, NT, preferred_element_type=f32)
        return c

    lax.fori_loop(0, S // TN1, p1, 0)

    cp_wo.wait()
    ri = lax.broadcasted_iota(jnp.int32, (D, D), 0).astype(f32)
    ci = lax.broadcasted_iota(jnp.int32, (D, D), 1).astype(f32)
    mask = _head_of(ri) == _head_of(ci)
    kvm = jnp.where(mask, kv_acc[...], 0.0).astype(bf16)
    m = jnp.dot(kvm, wo_v[...], preferred_element_type=f32)
    mT_v[...] = m.T.astype(bf16)
    zrow = z_acc[...].T
    zrow = jnp.sum(zrow, axis=0, keepdims=True)
    hi = lax.broadcasted_iota(jnp.int32, (H, D), 0).astype(f32)
    di = lax.broadcasted_iota(jnp.int32, (H, D), 1).astype(f32)
    zc_v[...] = jnp.where(hi == _head_of(di), zrow, 0.0).astype(bf16)
    di2 = lax.broadcasted_iota(jnp.int32, (D, 2 * H), 0).astype(f32)
    hi2 = lax.broadcasted_iota(jnp.int32, (D, 2 * H), 1)
    hi2 = jnp.where(hi2 >= H, hi2 - H, hi2).astype(f32)
    e_v[...] = jnp.where(_head_of(di2) == hi2, 1.0, 0.0).astype(bf16)

    cp_w1.wait()
    cp_w2.wait()

    def p2(i, c):
        c0 = pl.multiple_of(i * TN2, TN2)
        pq = pqT_v[:, pl.ds(c0, TN2)]
        den = jnp.dot(zc_v[...], pq, preferred_element_type=f32) + 1e-6
        rec = 1.0 / den
        rhi = rec.astype(bf16)
        rlo = (rec - rhi.astype(f32)).astype(bf16)
        rcat = jnp.concatenate([rhi, rlo], axis=0)
        rexp = jnp.dot(e_v[...], rcat, preferred_element_type=f32)
        pqs = (pq.astype(f32) * rexp).astype(bf16)
        attn = jnp.dot(mT_v[...], pqs, preferred_element_type=f32)
        h = xT_v[:, pl.ds(c0, TN2)].astype(f32) + attn
        hln = _lnT(h).T.astype(bf16)
        acc = h + b2c_v[:, 0:1]
        for f0 in range(0, F, FC):
            a = jnp.dot(hln, w1_v[:, f0:f0 + FC], preferred_element_type=f32) + b1_ref[:, f0:f0 + FC].astype(f32)
            a = jnp.maximum(a, 0.0)
            a = (a * a).astype(bf16)
            acc = acc + lax.dot_general(w2T_v[:, f0:f0 + FC], a, NT, preferred_element_type=f32)
        oT_v[:, pl.ds(c0, TN2)] = acc.astype(bf16)
        pltpu.make_async_copy(oT_v.at[:, pl.ds(c0, TN2)], oT_hbm.at[:, pl.ds(c0, TN2)], sems.at[5]).start()
        return c

    lax.fori_loop(0, S // TN2, p2, 0)
    pltpu.make_async_copy(oT_v, oT_hbm, sems.at[5]).wait()


@jax.jit
def pallas_sequential_preLN__linear_attn_block__dense_activation_squared_relu__prompt_kernel(
    A_x, A_wqkv, A_wo, B_x, B_w1, B_b1, B_w2, B_b2,
):
    xT = A_x.reshape(S, D).T
    w2T = B_w2.T
    b1 = B_b1.reshape(1, F)
    b2 = B_b2.reshape(1, D)
    hbm_spec = pl.BlockSpec(memory_space=pltpu.MemorySpace.HBM)
    vmem_spec = pl.BlockSpec(memory_space=pltpu.VMEM)
    outT = pl.pallas_call(
        _kernel,
        out_shape=jax.ShapeDtypeStruct((D, S), bf16),
        in_specs=[hbm_spec, hbm_spec, hbm_spec, hbm_spec, vmem_spec, hbm_spec, vmem_spec],
        out_specs=hbm_spec,
        scratch_shapes=[
            pltpu.VMEM((D, S), bf16),
            pltpu.VMEM((D, 3 * D), bf16),
            pltpu.VMEM((D, D), bf16),
            pltpu.VMEM((D, F), bf16),
            pltpu.VMEM((D, F), bf16),
            pltpu.VMEM((3 * D, D), bf16),
            pltpu.VMEM((D, S), bf16),
            pltpu.VMEM((D, D), f32),
            pltpu.VMEM((D, 128), f32),
            pltpu.VMEM((D, D), bf16),
            pltpu.VMEM((H, D), bf16),
            pltpu.VMEM((D, 2 * H), bf16),
            pltpu.VMEM((D, 128), f32),
            pltpu.VMEM((D, S), bf16),
            pltpu.SemaphoreType.DMA((6,)),
        ],
        compiler_params=pltpu.CompilerParams(vmem_limit_bytes=100 * 1024 * 1024),
    )(xT, A_wqkv, A_wo, B_w1, b1, w2T, b2)
    return outT.T.reshape(1, S, D)
```

```python
import jax
import jax.numpy as jnp
from jax import lax
import jax.experimental.pallas as pl
import jax.experimental.pallas.tpu as pltpu

S, D, F, H = 2048, 576, 4608, 32
DH = D // H
TN1 = 512
TN2 = 512
FC = 512
G = 72
NG = D // G
EPS = 1e-5
f32 = jnp.float32
bf16 = jnp.bfloat16
NT = (((1,), (1,)), ((), ()))
WCH = [(0, 128), (128, 128), (256, 128), (384, 128), (512, 64)]
NX = S // TN1


def _lnT(x):
    mu = jnp.mean(x, axis=0, keepdims=True)
    xc = x - mu
    var = jnp.mean(xc * xc, axis=0, keepdims=True)
    return xc * lax.rsqrt(var + EPS)


def _phi(t):
    return jnp.where(t > 0, t + 1.0, jnp.exp(t)) + 1e-6


def _head_of(idx_f32):
    return jnp.floor((idx_f32 + 0.5) * (1.0 / DH))


def _kernel(xT_hbm, wqkv_hbm, wo_hbm, w1_hbm, b1_ref, w2T_hbm, b2_ref, oT_hbm,
            xT_v, wqkv_v, wo_v, w1_v, w2T_v, wqkvT_v, pqT_v, kv_acc, z_acc, m_v, mT_v, zc_v, b2c_v, oT_v,
            sem_w, sem_x, sems):
    cp_wq = [pltpu.make_async_copy(wqkv_hbm.at[pl.ds(r, n), :], wqkv_v.at[pl.ds(r, n), :], sem_w.at[j])
             for j, (r, n) in enumerate(WCH)]

    def cp_x(i):
        return pltpu.make_async_copy(xT_hbm.at[:, pl.ds(i * TN1, TN1)], xT_v.at[:, pl.ds(i * TN1, TN1)],
                                     sem_x.at[i])

    cp_wo = pltpu.make_async_copy(wo_hbm, wo_v, sems.at[0])
    cp_w1 = pltpu.make_async_copy(w1_hbm, w1_v, sems.at[1])
    cp_w2 = pltpu.make_async_copy(w2T_hbm, w2T_v, sems.at[2])
    for c in cp_wq:
        c.start()
    cp_x(0).start()

    kv_acc[...] = jnp.zeros_like(kv_acc)
    z_acc[...] = jnp.zeros_like(z_acc)
    b2c_v[...] = jnp.broadcast_to(b2_ref[...].astype(f32).reshape(1, D), (128, D)).T

    for j, (r, n) in enumerate(WCH):
        cp_wq[j].wait()
        wqkvT_v[:, r:r + n] = wqkv_v[r:r + n, :].astype(f32).T.astype(bf16)
    for i in range(1, NX):
        cp_x(i).start()
    cp_wo.start()
    cp_w1.start()
    cp_w2.start()

    def p1(i, c):
        c0 = pl.multiple_of(i * TN1, TN1)
        pltpu.make_async_copy(xT_hbm.at[:, pl.ds(c0, TN1)], xT_v.at[:, pl.ds(c0, TN1)], sem_x.at[i]).wait()
        x = xT_v[:, pl.ds(c0, TN1)].astype(f32)
        xln = _lnT(x).astype(bf16)
        qkvT = jnp.dot(wqkvT_v[...], xln, preferred_element_type=f32)
        pqT_v[:, pl.ds(c0, TN1)] = _phi(qkvT[0:D]).astype(bf16)
        pkT = _phi(qkvT[D:2 * D])
        zs = pkT[:, 0:128]
        for j in range(1, TN1 // 128):
            zs = zs + pkT[:, j * 128:(j + 1) * 128]
        z_acc[...] += zs
        for g in range(NG):
            pk_g = pkT[g * G:(g + 1) * G].astype(bf16)
            v_g = qkvT[2 * D + g * G:2 * D + (g + 1) * G].astype(bf16)
            kv_acc[g] += lax.dot_general(pk_g, v_g, NT, preferred_element_type=f32)
        return c

    lax.fori_loop(0, NX, p1, 0)

    cp_wo.wait()
    ri = lax.broadcasted_iota(jnp.int32, (G, G), 0).astype(f32)
    ci = lax.broadcasted_iota(jnp.int32, (G, G), 1).astype(f32)
    mask = _head_of(ri) == _head_of(ci)
    wo32 = wo_v[...].astype(f32)
    for g in range(NG):
        kvm = jnp.where(mask, kv_acc[g], 0.0).astype(bf16)
        m_v[g * G:(g + 1) * G, :] = jnp.dot(kvm, wo32[g * G:(g + 1) * G].astype(bf16),
                                            preferred_element_type=f32)
    mT_v[...] = m_v[...].T.astype(bf16)
    zrow = z_acc[...].T
    zrow = jnp.sum(zrow, axis=0, keepdims=True)
    hi = lax.broadcasted_iota(jnp.int32, (H, D), 0).astype(f32)
    di = lax.broadcasted_iota(jnp.int32, (H, D), 1).astype(f32)
    zc_v[...] = jnp.where(hi == _head_of(di), zrow, 0.0).astype(bf16)

    cp_w1.wait()
    cp_w2.wait()
    b1row = b1_ref[...].astype(f32).reshape(1, F)

    def p2(i, c):
        c0 = pl.multiple_of(i * TN2, TN2)
        pq = pqT_v[:, pl.ds(c0, TN2)]
        den = jnp.dot(zc_v[...], pq, preferred_element_type=f32) + 1e-6
        rec = 1.0 / den
        rexp = jnp.concatenate([jnp.broadcast_to(rec[hh:hh + 1, :], (DH, TN2)) for hh in range(H)], axis=0)
        pqs = (pq.astype(f32) * rexp).astype(bf16)
        attn = jnp.dot(mT_v[...], pqs, preferred_element_type=f32)
        h = xT_v[:, pl.ds(c0, TN2)].astype(f32) + attn
        hln = _lnT(h).T.astype(bf16)
        acc = h + b2c_v[:, 0:1]
        for f0 in range(0, F, FC):
            a = jnp.dot(hln, w1_v[:, f0:f0 + FC], preferred_element_type=f32) + b1row[:, f0:f0 + FC]
            a = jnp.maximum(a, 0.0)
            a = (a * a).astype(bf16)
            acc = acc + lax.dot_general(w2T_v[:, f0:f0 + FC], a, NT, preferred_element_type=f32)
        oT_v[:, pl.ds(c0, TN2)] = acc.astype(bf16)
        pltpu.make_async_copy(oT_v.at[:, pl.ds(c0, TN2)], oT_hbm.at[:, pl.ds(c0, TN2)], sems.at[3]).start()
        return c

    lax.fori_loop(0, S // TN2, p2, 0)
    pltpu.make_async_copy(oT_v, oT_hbm, sems.at[3]).wait()


@jax.jit
def pallas_sequential_preLN__linear_attn_block__dense_activation_squared_relu__prompt_kernel(
    A_x: jax.Array,
    A_wqkv: jax.Array,
    A_wo: jax.Array,
    B_x: jax.Array,
    B_w1: jax.Array,
    B_b1: jax.Array,
    B_w2: jax.Array,
    B_b2: jax.Array,
):
    del B_x
    xT = A_x.reshape(S, D).T
    w2T = B_w2.T
    hbm_spec = pl.BlockSpec(memory_space=pltpu.MemorySpace.HBM)
    vmem_spec = pl.BlockSpec(memory_space=pltpu.VMEM)
    outT = pl.pallas_call(
        _kernel,
        out_shape=jax.ShapeDtypeStruct((D, S), bf16),
        in_specs=[hbm_spec, hbm_spec, hbm_spec, hbm_spec, vmem_spec, hbm_spec, vmem_spec],
        out_specs=hbm_spec,
        scratch_shapes=[
            pltpu.VMEM((D, S), bf16),
            pltpu.VMEM((D, 3 * D), bf16),
            pltpu.VMEM((D, D), bf16),
            pltpu.VMEM((D, F), bf16),
            pltpu.VMEM((D, F), bf16),
            pltpu.VMEM((3 * D, D), bf16),
            pltpu.VMEM((D, S), bf16),
            pltpu.VMEM((NG, G, G), f32),
            pltpu.VMEM((D, 128), f32),
            pltpu.VMEM((D, D), f32),
            pltpu.VMEM((D, D), bf16),
            pltpu.VMEM((H, D), bf16),
            pltpu.VMEM((D, 128), f32),
            pltpu.VMEM((D, S), bf16),
            pltpu.SemaphoreType.DMA((len(WCH),)),
            pltpu.SemaphoreType.DMA((NX,)),
            pltpu.SemaphoreType.DMA((4,)),
        ],
        compiler_params=pltpu.CompilerParams(vmem_limit_bytes=100 * 1024 * 1024),
    )(xT, A_wqkv, A_wo, B_w1, B_b1, w2T, B_b2)
    return outT.T.reshape(1, S, D)
```

```python
import jax
import jax.numpy as jnp
from jax import lax
import jax.experimental.pallas as pl
import jax.experimental.pallas.tpu as pltpu

S, D, F, H = 2048, 576, 4608, 32
DH = D // H
TN1 = 512
TN2 = 512
FC = 512
G = 72
NG = D // G
EPS = 1e-5
f32 = jnp.float32
bf16 = jnp.bfloat16
NT = (((1,), (1,)), ((), ()))
WCH = [(0, 128), (128, 128), (256, 128), (384, 128), (512, 64)]
NX = S // TN1


def _lnT(x):
    mu = jnp.mean(x, axis=0, keepdims=True)
    xc = x - mu
    var = jnp.mean(xc * xc, axis=0, keepdims=True)
    return xc * lax.rsqrt(var + EPS)


def _phi(t):
    return jnp.where(t > 0, t + 1.0, jnp.exp(t)) + 1e-6


def _head_of(idx_f32):
    return jnp.floor((idx_f32 + 0.5) * (1.0 / DH))


def _kernel(xT_hbm, wqkv_hbm, wo_hbm, w1_hbm, b1_ref, w2T_hbm, b2_ref, oT_hbm,
            xT_v, wqkv_v, wo_v, w1_v, w2T_v, wqkvT_v, pqT_v, kv_acc, z_acc, m_v, mT_v, zc_v, b2c_v, oT_v,
            sem_w, sem_x, sems):
    cp_wq = [pltpu.make_async_copy(wqkv_hbm.at[pl.ds(r, n), :], wqkv_v.at[pl.ds(r, n), :], sem_w.at[j])
             for j, (r, n) in enumerate(WCH)]

    def cp_x(i):
        return pltpu.make_async_copy(xT_hbm.at[:, pl.ds(i * TN1, TN1)], xT_v.at[:, pl.ds(i * TN1, TN1)],
                                     sem_x.at[i])

    cp_wo = pltpu.make_async_copy(wo_hbm, wo_v, sems.at[0])
    cp_w1 = pltpu.make_async_copy(w1_hbm, w1_v, sems.at[1])
    cp_w2 = pltpu.make_async_copy(w2T_hbm, w2T_v, sems.at[2])
    for c in cp_wq:
        c.start()
    cp_x(0).start()

    kv_acc[...] = jnp.zeros_like(kv_acc)
    z_acc[...] = jnp.zeros_like(z_acc)
    b2c_v[...] = jnp.broadcast_to(b2_ref[...].astype(f32).reshape(1, D), (128, D)).T

    for j, (r, n) in enumerate(WCH):
        cp_wq[j].wait()
        wqkvT_v[:, r:r + n] = wqkv_v[r:r + n, :].astype(f32).T.astype(bf16)
    for i in range(1, NX):
        cp_x(i).start()
    cp_wo.start()
    cp_w1.start()
    cp_w2.start()

    def p1(i, c):
        c0 = pl.multiple_of(i * TN1, TN1)
        pltpu.make_async_copy(xT_hbm.at[:, pl.ds(c0, TN1)], xT_v.at[:, pl.ds(c0, TN1)], sem_x.at[i]).wait()
        x = xT_v[:, pl.ds(c0, TN1)].astype(f32)
        xln = _lnT(x).astype(bf16)
        qkvT = jnp.dot(wqkvT_v[...], xln, preferred_element_type=f32)
        pqT_v[:, pl.ds(c0, TN1)] = _phi(qkvT[0:D]).astype(bf16)
        pkT = _phi(qkvT[D:2 * D])
        zs = pkT[:, 0:128]
        for j in range(1, TN1 // 128):
            zs = zs + pkT[:, j * 128:(j + 1) * 128]
        z_acc[...] += zs
        for g in range(NG):
            pk_g = pkT[g * G:(g + 1) * G].astype(bf16)
            v_g = qkvT[2 * D + g * G:2 * D + (g + 1) * G].astype(bf16)
            kv_acc[g] += lax.dot_general(pk_g, v_g, NT, preferred_element_type=f32)
        return c

    lax.fori_loop(0, NX, p1, 0)

    cp_wo.wait()
    ri = lax.broadcasted_iota(jnp.int32, (G, G), 0).astype(f32)
    ci = lax.broadcasted_iota(jnp.int32, (G, G), 1).astype(f32)
    mask = _head_of(ri) == _head_of(ci)
    wo32 = wo_v[...].astype(f32)
    for g in range(NG):
        kvm = jnp.where(mask, kv_acc[g], 0.0).astype(bf16)
        m_v[g * G:(g + 1) * G, :] = jnp.dot(kvm, wo32[g * G:(g + 1) * G].astype(bf16),
                                            preferred_element_type=f32)
    mT_v[...] = m_v[...].T.astype(bf16)
    zrow = z_acc[...].T
    zrow = jnp.sum(zrow, axis=0, keepdims=True)
    hi = lax.broadcasted_iota(jnp.int32, (H, D), 0).astype(f32)
    di = lax.broadcasted_iota(jnp.int32, (H, D), 1).astype(f32)
    zc_v[...] = jnp.where(hi == _head_of(di), zrow, 0.0).astype(bf16)

    cp_w1.wait()
    cp_w2.wait()
    b1row = b1_ref[...].astype(f32).reshape(1, F)

    def p2(i, c):
        c0 = pl.multiple_of(i * TN2, TN2)
        pq = pqT_v[:, pl.ds(c0, TN2)]
        den = jnp.dot(zc_v[...], pq, preferred_element_type=f32) + 1e-6
        rec = 1.0 / den
        rexp = jnp.concatenate([jnp.broadcast_to(rec[hh:hh + 1, :], (DH, TN2)) for hh in range(H)], axis=0)
        pqs = (pq.astype(f32) * rexp).astype(bf16)
        attn = jnp.dot(mT_v[...], pqs, preferred_element_type=f32)
        h = xT_v[:, pl.ds(c0, TN2)].astype(f32) + attn
        hln = _lnT(h).T.astype(bf16)
        acc = h + b2c_v[:, 0:1]
        for f0 in range(0, F, FC):
            a = jnp.dot(hln, w1_v[:, f0:f0 + FC], preferred_element_type=f32) + b1row[:, f0:f0 + FC]
            a = jnp.maximum(a, 0.0)
            a = (a * a).astype(bf16)
            acc = acc + lax.dot_general(w2T_v[:, f0:f0 + FC], a, NT, preferred_element_type=f32)
        HW = TN2 // 4
        for hh in range(4):
            ch = pl.multiple_of(c0 + hh * HW, HW)
            oT_v[:, pl.ds(ch, HW)] = acc[:, hh * HW:(hh + 1) * HW].astype(bf16)
            pltpu.make_async_copy(oT_v.at[:, pl.ds(ch, HW)], oT_hbm.at[:, pl.ds(ch, HW)], sems.at[3]).start()
        return c

    lax.fori_loop(0, S // TN2, p2, 0)
    pltpu.make_async_copy(oT_v, oT_hbm, sems.at[3]).wait()


@jax.jit
def pallas_sequential_preLN__linear_attn_block__dense_activation_squared_relu__prompt_kernel(
    A_x: jax.Array,
    A_wqkv: jax.Array,
    A_wo: jax.Array,
    B_x: jax.Array,
    B_w1: jax.Array,
    B_b1: jax.Array,
    B_w2: jax.Array,
    B_b2: jax.Array,
):
    del B_x
    xT = A_x.reshape(S, D).T
    w2T = B_w2.T
    hbm_spec = pl.BlockSpec(memory_space=pltpu.MemorySpace.HBM)
    vmem_spec = pl.BlockSpec(memory_space=pltpu.VMEM)
    outT = pl.pallas_call(
        _kernel,
        out_shape=jax.ShapeDtypeStruct((D, S), bf16),
        in_specs=[hbm_spec, hbm_spec, hbm_spec, hbm_spec, vmem_spec, hbm_spec, vmem_spec],
        out_specs=hbm_spec,
        scratch_shapes=[
            pltpu.VMEM((D, S), bf16),
            pltpu.VMEM((D, 3 * D), bf16),
            pltpu.VMEM((D, D), bf16),
            pltpu.VMEM((D, F), bf16),
            pltpu.VMEM((D, F), bf16),
            pltpu.VMEM((3 * D, D), bf16),
            pltpu.VMEM((D, S), bf16),
            pltpu.VMEM((NG, G, G), f32),
            pltpu.VMEM((D, 128), f32),
            pltpu.VMEM((D, D), f32),
            pltpu.VMEM((D, D), bf16),
            pltpu.VMEM((H, D), bf16),
            pltpu.VMEM((D, 128), f32),
            pltpu.VMEM((D, S), bf16),
            pltpu.SemaphoreType.DMA((len(WCH),)),
            pltpu.SemaphoreType.DMA((NX,)),
            pltpu.SemaphoreType.DMA((4,)),
        ],
        compiler_params=pltpu.CompilerParams(vmem_limit_bytes=100 * 1024 * 1024),
    )(xT, A_wqkv, A_wo, B_w1, B_b1, w2T, B_b2)
    return outT.T.reshape(1, S, D)
```
